```python
import os as _os
_os.environ.setdefault("JAX_PLATFORMS", "cpu")
import jax
import jax.numpy as jnp

def _softmax(x, axis=-1):
    return jax.nn.softmax(x, axis=axis)
def _gelu(x):
    return jax.nn.gelu(x, approximate=True)
def _silu(x):
    return jax.nn.silu(x)
def _sigmoid(x):
    return jax.nn.sigmoid(x)
def _layernorm(x, axis=-1, eps=1e-5):
    m = jnp.mean(x, axis=axis, keepdims=True)
    v = jnp.var(x, axis=axis, keepdims=True)
    return (x - m) / jnp.sqrt(v + eps)
def _scatter_add(tgt, idx, src, axis=0):
    return tgt.at[idx].add(src)
def _segment_sum(src, seg, n):
    return jax.ops.segment_sum(src, seg, n)
class _Rng:
    def __init__(self, key):
        self._k = key
    def _next(self):
        self._k, sub = jax.random.split(self._k)
        return sub
    def normal(self, shape):
        return jax.random.normal(self._next(), shape, dtype=jnp.bfloat16)
    def randint(self, lo, hi, shape):
        return jax.random.randint(self._next(), shape, lo, hi, dtype=jnp.int32)
    def uniform(self, shape, lo=0.0, hi=1.0):
        return jax.random.uniform(self._next(), shape, jnp.bfloat16, lo, hi)
    def permutation(self, n):
        return jax.random.permutation(self._next(), n)


kernel_name = 'concat_heads__ssm_conv_h3__sliding_block__prompt'

def setup_inputs():
    _rng = _Rng(jax.random.key(int.from_bytes(__import__("os").urandom(4), "little")))
    _w = (lambda a: (lambda t: t.astype(jnp.bfloat16) if jnp.issubdtype(t.dtype, jnp.floating) else t)(jnp.asarray(a)))
    def _A_setup():
        B, S, D = 1, 2048, 512
        ks = 4
        return {
            "q": _w((lambda *s: _rng.normal(s) * 0.05)(B, S, D)),
            "k": _w((lambda *s: _rng.normal(s) * 0.2)(B, S, D)),
            "v": _w((lambda *s: _rng.normal(s) * 0.2)(B, S, D)),
            "shift_k": _w((lambda *s: _rng.normal(s) * 0.2)(D, ks) * 0.5),
            "ssm_k": _w((lambda *s: _rng.normal(s) * 0.2)(D, S) * (1.0 / S ** 0.5)),
            "ssm_D": _w((lambda *s: _rng.normal(s) * 0.2)(D)),
        }
    _A_in = _A_setup()

    def _B_setup():
        B, S, D = 1, 2048, 512
        return {
            "x": _w((lambda *s: _rng.normal(s) * 0.2)(B, S, D)),
            "wqkv": _w((lambda *s: _rng.normal(s) * 0.2)(D, 3 * D)),
            "wo": _w((lambda *s: _rng.normal(s) * 0.05)(D, D)),
        }
    _B_in = _B_setup()

    return {
        "A_q": _A_in["q"],
        "A_k": _A_in["k"],
        "A_v": _A_in["v"],
        "A_shift_k": _A_in["shift_k"],
        "A_ssm_k": _A_in["ssm_k"],
        "A_ssm_D": _A_in["ssm_D"],
        "B_x": _B_in["x"],
        "B_wqkv": _B_in["wqkv"],
        "B_wo": _B_in["wo"],
    }

def reference(A_q, A_k, A_v, A_shift_k, A_ssm_k, A_ssm_D, B_x, B_wqkv, B_wo):
    def _A_ref(q, k, v, shift_k, ssm_k, ssm_D):
        B, S, D = q.shape
        ks = shift_k.shape[-1]
        k_pad = jnp.pad(k, ((0, 0), (ks - 1, 0), (0, 0)))
        k_shift = jnp.zeros_like(k)
        for t in range(ks):
            k_shift = k_shift + k_pad[:, t:t + S, :] * shift_k[:, ks - 1 - t][None, None, :]
        kv = k_shift * v
        L = 2 * S
        kv_pad = jnp.pad(kv, ((0, 0), (0, S), (0, 0)))
        kf_pad = jnp.pad(ssm_k, ((0, 0), (0, S)))
        kv_f = (lambda x, axes=(-2,-1): jnp.fft.rfft2(x.astype(jnp.float32), axes=axes))(kv_pad[:, None, :, :], axes=(1, 2))
        kf_f = (lambda x, axes=(-2,-1): jnp.fft.rfft2(x.astype(jnp.float32), axes=axes))(kf_pad[:, None, :], axes=(1, 2))
        kf_f = (lambda x, *d: x.transpose(*d))(kf_f, 1, 2, 0)
        y_f = kv_f * kf_f[None, :, :, :]
        y = (lambda x, s, axes=(-2,-1): jnp.fft.irfft2(x, s=s, axes=axes).astype(jnp.bfloat16))(y_f, (1, L), axes=(1, 2))[:, 0, :S, :]
        y = y + kv * ssm_D[None, None, :]
        return q * y

    def _B_ref(x, wqkv, wo):
        B, S, D = x.shape
        H = 32; Dh = D // H; W = 256
        qkv = (lambda x, *d: x.transpose(*d))((x @ wqkv).reshape(B, S, 3, H, Dh), 2, 0, 3, 1, 4)
        q, k, v = qkv[0], qkv[1], qkv[2]
        scores = jnp.einsum("bhqd,bhkd->bhqk", q, k) * (Dh ** -0.5)
        idx = jnp.arange(S)
        mask = (idx[:, None] - idx[None, :] >= 0) & (idx[:, None] - idx[None, :] < W)
        scores = jnp.where(mask[None, None], scores, -1e9)
        p = _softmax(scores, axis=-1)
        o = jnp.einsum("bhqk,bhkd->bhqd", p, v)
        return (lambda x, *d: x.transpose(*d))(o, 0, 2, 1, 3).reshape(B, S, D) @ wo

    a = _A_ref(A_q, A_k, A_v, A_shift_k, A_ssm_k, A_ssm_D)
    b = _B_ref(B_x, B_wqkv, B_wo)
    return jnp.concatenate([a, b], axis=-1)
```

```python
import jax, jax.numpy as jnp, numpy as np, ml_dtypes
from jax import lax
from jax.experimental import pallas as pl
from jax.experimental.pallas import tpu as pltpu
S=2048; D=512
f32=jnp.float32; bf16=jnp.bfloat16
NT=(((1,),(1,)),((),()))
N1=32;N2=64
def consts():
    k1=np.arange(N1)[:,None]; n1=np.arange(N1)[None,:]
    w=np.exp(1j*np.pi*(4*k1+1)*n1/(2*N1))
    F1=np.concatenate([w.real,w.imag],0)
    k2=np.arange(N2)[None,:,None]; n2=np.arange(N2)[None,None,:]; kk=np.arange(N1)[:,None,None]
    w=np.exp(1j*np.pi*(4*kk+1)*n2/(2*S)+2j*np.pi*k2*n2/N2)
    F2=np.concatenate([np.concatenate([w.real,-w.imag],2),np.concatenate([w.imag,w.real],2)],1)
    G2=F2.transpose(0,2,1); G1=F1.T/S
    return [np.ascontiguousarray(a).astype(ml_dtypes.bfloat16) for a in (F1,F2,G2,G1)]
F1c,F2c,G2c,G1c=consts()
PAD=1
class W128:
    def __init__(s,ref,n): s.ref=ref; s.n=n
    def _p(s,i):
        return (i[0],4) if isinstance(i,tuple) else (i,s.n)
    def __getitem__(s,i):
        i,n=s._p(i)
        return jnp.concatenate([s.ref[c,i,:] for c in range(n)],axis=1)
    def __setitem__(s,i,v):
        i,n=s._p(i)
        for c in range(n): s.ref[c,i,:]=v[:,c*128:(c+1)*128]
NEG=-1e30
def part_a(q_ref,k_ref,v_ref,sk_ref,h_ref,d_ref,F1,F2,G2,G1,oa,kf,kv,ht,B,oA):
    kv=W128(kv,4);ht=W128(ht,4);B=W128(B,8)
    kf[:,0:8,:]=jnp.zeros((4,8,128),f32); dd=d_ref[...].astype(f32).reshape(1,D)
    skT=sk_ref[...].astype(f32)
    eye=(lax.broadcasted_iota(jnp.int32,(128,128),0)==lax.broadcasted_iota(jnp.int32,(128,128),1)).astype(bf16)
    RB=128
    def p0(i,c):
        r0=pl.multiple_of(i*RB,RB)
        for u in range(2):
            r1=r0+64*u
            for cc in range(4):
                sl=slice(cc*128,cc*128+128)
                k0=k_ref[pl.ds(r1,64),sl].astype(f32)
                kf[cc,pl.ds(r1+8,64),:]=k0
                ks=k0*skT[0:1,sl]
                for t in range(1,4): ks=ks+kf[cc,pl.ds(r1+8-t,64),:]*skT[t:t+1,sl]
                kv.ref[cc,pl.ds((2*i+u)*65,64),:]=ks*v_ref[pl.ds(r1,64),sl].astype(f32)
        hh=lax.dot_general(eye,h_ref[:,pl.ds(r0,RB)],NT,preferred_element_type=f32)
        for u in range(2):
            ht[pl.ds((2*i+u)*65,64)]=hh[u*64:u*64+64]
        return c
    yield p0
    U=8
    ST=128+PAD
    def s1(i,c):
        for u in range(U):
            n2=i*U+u
            X=jnp.concatenate([kv[pl.ds(n2,N1,stride=65)],ht[pl.ds(n2,N1,stride=65)]],axis=1).astype(bf16)
            A=jnp.dot(F1[...],X,preferred_element_type=f32)
            B[pl.ds(n2,N1,stride=ST)]=A[:N1]
            B[pl.ds(n2+N2,N1,stride=ST)]=A[N1:]
        return c
    lax.fori_loop(0,N2//U,s1,0)
    def s2(i,c):
        Ys={}
        for u in range(5):
            if u<4:
                k1=i*4+u
                W=jnp.dot(F2[k1],B[pl.ds(k1*ST,128)].astype(bf16),preferred_element_type=f32)
            if u>0:
                k0=i*4+u-1
                B[pl.ds(k0*ST,128),0:D]=jnp.dot(G2[k0],Ys[u-1],preferred_element_type=f32)
            if u<4:
                ur,ui,hr,hi=W[:64,:D],W[64:,:D],W[:64,D:],W[64:,D:]
                Ys[u]=jnp.concatenate([ur*hr-ui*hi,ur*hi+ui*hr],axis=0).astype(bf16)
        return c
    lax.fori_loop(0,N1//4,s2,0)
    def s3(i,c):
        for u in range(U):
            n2=i*U+u
            Z=jnp.concatenate([B[pl.ds(n2,N1,stride=ST),0:D],B[pl.ds(n2+N2,N1,stride=ST),0:D]],axis=0).astype(bf16)
            ht[pl.ds(n2,N1,stride=65)]=jnp.dot(G1[...],Z,preferred_element_type=f32)
        return c
    lax.fori_loop(0,N2//U,s3,0)
    def p4(i,c):
        r0=pl.multiple_of(i*RB,RB)
        g=lambda r:jnp.concatenate([r[pl.ds((2*i+u)*65,64)] for u in range(2)],axis=0)
        y=g(ht)+g(kv)*dd
        oa[pl.ds(r0,RB)]=(q_ref[pl.ds(r0,RB)].astype(f32)*y).astype(bf16)
        oA(r0).start()
        return c
    lax.fori_loop(0,S//RB,p4,0)
def part_b(x_ref,w_ref,wo_ref,ob,wqT,wvT,ka,kb,vt0,vt1,cp,xc,oB,p0,w3):
    cp['wv'].wait();cp['wk'].wait()
    wvT[...] = (w_ref[:, 2*D:3*D].astype(f32)).T.astype(bf16)
    z = jnp.zeros((256, D), bf16)
    ka[0:256] = z; kb[0:256] = z
    vt0[:, 0:256] = jnp.zeros((D,256), bf16); vt1[:, 0:256] = jnp.zeros((D,256), bf16)
    vt1[:, S+128:S+256] = jnp.zeros((D,128), bf16)
    ka[S+192:S+256] = jnp.zeros((64,D), bf16); kb[S+192:S+256] = jnp.zeros((64,D), bf16)
    for i in range(2,8): xc(i).start()
    cp['wq'].start();cp['wo'].start()
    PB=256
    odd = ((lax.broadcasted_iota(jnp.int32, (PB, D), 1) >> 4) & 1) == 1
    lane = lax.broadcasted_iota(jnp.int32, (D, 128), 1)
    def proj(i, c):
        r0 = pl.multiple_of(i*PB, PB)
        xc(i).wait()
        xb = x_ref[pl.ds(r0, PB), :]
        k = jnp.dot(xb, w_ref[:, D:2*D], preferred_element_type=f32)
        pa=jnp.concatenate([ka[pl.ds(r0+192,64),:].astype(f32),k[:PB-64]],axis=0)
        pb=jnp.concatenate([kb[pl.ds(r0+192,64),:].astype(f32),k[:PB-64]],axis=0)
        ka[pl.ds(r0+192,PB),:]=jnp.where(odd,k,pa).astype(bf16)
        kb[pl.ds(r0+192,PB),:]=jnp.where(odd,pb,k).astype(bf16)
        ka[pl.ds(r0+192+PB,64),:]=k[PB-64:].astype(bf16); kb[pl.ds(r0+192+PB,64),:]=k[PB-64:].astype(bf16)
        vT = lax.dot_general(wvT[...], xb, NT, preferred_element_type=f32)
        vt0[:, pl.ds(r0+256, PB)] = vT.astype(bf16)
        for t in range(PB//128):
            vr = pltpu.roll(vT[:, t*128:(t+1)*128], 64, 1).astype(bf16)
            c0 = r0 + 128 + t*128
            p0 = vt1[:, pl.ds(c0, 128)]
            vt1[:, pl.ds(c0, 128)] = jnp.where(lane >= 64, vr, p0)
            vt1[:, pl.ds(c0+128, 128)] = vr
        return c
    lax.fori_loop(0, S//PB, proj, 0)
    cp['wq'].wait();cp['wo'].wait()
    for c in w3: c.start()
    wqT[...] = (w_ref[:, 0:D].astype(f32)).T.astype(bf16)
    l16 = lax.broadcasted_iota(jnp.int32, (16,128), 1)
    lo16 = l16 < 64
    rr = lax.broadcasted_iota(jnp.int32, (64,128), 0)
    ll = lax.broadcasted_iota(jnp.int32, (64,128), 1) & 63
    tri = ll < rr
    def qblock(j, first, NB):
        R=[pl.multiple_of((j+b)*128,128) for b in range(NB)]
        QT={}
        def qp(b):
            QT[b]=(lax.dot_general(wqT[...], x_ref[pl.ds(R[b],128),:], NT, preferred_element_type=f32) * (0.25*np.log2(np.e))).astype(bf16)
        qp(0)
        row = lax.broadcasted_iota(jnp.int32, (320,128), 0)
        hl = lax.broadcasted_iota(jnp.int32, (320,128), 1) & 64
        valid=[(row+hl+128*b)>=256 for b in range(NB)]
        z16 = jnp.zeros((16,128), bf16)
        steps=[(G,arr,b) for b in range(NB) for G in range(4) for arr in range(2)]
        def mkW(G,arr,bb):
            qT=QT[bb]
            Ws=[]
            for p in range(4):
                ha = G*128 + p*32
                qa = qT[ha:ha+16]; qb = qT[ha+16:ha+32]
                if arr == 0:
                    wa = jnp.where(lo16, qa, z16); wb = jnp.where(lo16, z16, qb)
                else:
                    wa = jnp.where(lo16, z16, qa); wb = jnp.where(lo16, qb, z16)
                Ws.append(jnp.concatenate([z16]*(2*p) + [wa, wb] + [z16]*(6-2*p), axis=0))
            return jnp.concatenate(Ws, axis=1)
        CH=[(0,64),(64,128),(128,192),(192,256)]
        tri4=jnp.concatenate([tri]*4,axis=1)
        def qk(t,c,W):
            G,arr,bb=steps[t]; r0=R[bb]; kr=(ka,kb)[arr]
            a,b=CH[c]
            def sc(a,b):
                s=jnp.dot(kr[pl.ds(r0+a,b-a), G*128:(G+1)*128], W, preferred_element_type=f32)
                if first:
                    s=jnp.where(jnp.concatenate([valid[bb][a:b]]*4,axis=1), s, NEG)
                return s
            if c==0:
                s=jnp.where(tri4, sc(0,64), sc(256,320))
            else:
                s=sc(a,b)
            SV[(t,c)] = s
            return jnp.max(s.reshape((b-a)//8,8,512),axis=0)
        def expv(t,p,m):
            G,arr,bb=steps[t]; r0=R[bb]
            ha = G*128 + p*32
            sl=slice(p*128,(p+1)*128)
            e=[jnp.exp2(SV[(t,c)][:,sl]-m[:,sl]) for c in range(4)]
            l=jnp.sum((e[0]+e[1])+(e[2]+e[3]),axis=0,keepdims=True)
            P=jnp.concatenate([jnp.where(tri,e[0],0.0),e[1],e[2],e[3],jnp.where(tri,0.0,e[0])],axis=0).astype(bf16)
            va = (vt0, vt1)[arr][ha:ha+16, pl.ds(r0, 384)]
            vb = (vt1, vt0)[arr][ha+16:ha+32, pl.ds(r0, 384)]
            vv = jnp.concatenate([va, vb], axis=0)[:, :320]
            return lambda: jnp.dot(vv, P, preferred_element_type=f32) * (1.0/l)
        def pv(t,p,l):
            G,arr,bb=steps[t]; r0=R[bb]
            ha = G*128 + p*32
            va = (vt0, vt1)[arr][ha:ha+16, pl.ds(r0, 384)]
            vb = (vt1, vt0)[arr][ha+16:ha+32, pl.ds(r0, 384)]
            vv = jnp.concatenate([va, vb], axis=0)[:, :320]
            return jnp.dot(vv, jnp.concatenate([PV[(t,c)][:,p*128:(p+1)*128] for c in range(5)],axis=0), preferred_element_type=f32) * l[:,p*128:(p+1)*128]
        SV={};PV={};res={}; ms={}; ls={}
        def fin(b):
            outs=[]
            for G in range(4):
                for p in range(4):
                    A=res[(8*b+2*G,p)]; B=res[(8*b+2*G+1,p)]
                    outs.append(jnp.where(lo16, A[0:16], B[0:16]))
                    outs.append(jnp.where(lo16, B[16:32], A[16:32]))
            if not first: p0(j+b-2,0)
            o = jnp.concatenate(outs, axis=0).T.astype(bf16)
            ob[pl.ds(R[b],128), :] = jnp.dot(o, wo_ref[...], preferred_element_type=f32).astype(bf16)
            oB(R[b]).start()
        for t in range(len(steps)+2):
            if t%8==6 and t//8+1<NB: qp(t//8+1)
            if t%8==3 and t>8: fin(t//8-1)
            if t<len(steps): W=mkW(*steps[t])
            macc=None; lacc=None
            for c in range(4):
                if t<len(steps):
                    mm=qk(t,c,W); macc = mm if macc is None else jnp.maximum(macc,mm)
                if 0<=t-1<len(steps): PV[(t-1,c)]=expv(t-1,c,ms[t-1])
                if t>=2: res[(t-2,c)]=PV[(t-2,c)]()
            if macc is not None: ms[t]=jnp.max(macc,axis=0,keepdims=True)
            if lacc is not None: ls[t-1]=1.0/jnp.sum(lacc,axis=0,keepdims=True)
        fin(NB-1)
    qblock(0,True,2)
    for c in w3[:3]: c.wait()
    def b2(i,c):
        qblock(2+i*2,False,2); return c
    lax.fori_loop(0,7,b2,0)
    lax.fori_loop(14,16,p0,0)

def kern(sk,d,F1,G1,qh,kh,vh,hh,xh,wh,woh,F2h,G2h,out,
         q,k,v,h,x,w,wo,F2,G2,oa,ob,kf,kv,ht,B,wqT,wvT,ka,kb,vt0,vt1,sem,xsem,osem):
    mk=pltpu.make_async_copy
    def wc(i,s): return mk(wh.at[:,i*D:(i+1)*D],w.at[:,i*D:(i+1)*D],sem.at[s])
    cp=dict(wv=wc(2,0),wk=wc(1,1),wq=wc(0,2),wo=mk(woh,wo,sem.at[3]))
    rest=[mk(a,b,sem.at[4+i]) for i,(a,b) in enumerate([(kh,k),(vh,v),(hh,h),(F2h,F2),(G2h,G2),(qh,q)])]
    xc=lambda i: mk(xh.at[pl.ds(i*256,256)],x.at[pl.ds(i*256,256)],xsem.at[i])
    cp['wv'].start();cp['wk'].start()
    for i in range(2): xc(i).start()
    oA=lambda r: mk(oa.at[pl.ds(r,128)],out.at[pl.ds(r,128),0:D],osem.at[0])
    oB=lambda r: mk(ob.at[pl.ds(r,128)],out.at[pl.ds(r,128),D:2*D],osem.at[1])
    ga=part_a(q,k,v,sk,h,d,F1,F2,G2,G1,oa,kf,kv,ht,B,oA)
    part_b(x,w,wo,ob,wqT,wvT,ka,kb,vt0,vt1,cp,xc,oB,next(ga),rest)
    for c in rest[3:]: c.wait()
    next(ga,None)
    mk(oa,oa,osem.at[0]).wait()
    mk(ob,ob,osem.at[1]).wait()

@jax.jit
def pallas_concat_heads__ssm_conv_h3__sliding_block__prompt_kernel(A_q,A_k,A_v,A_shift_k,A_ssm_k,A_ssm_D,B_x,B_wqkv,B_wo):
    V=pltpu.VMEM
    sc=[V((S,D),bf16)]*3+[V((D,S),bf16),V((S,D),bf16),V((D,3*D),bf16),V((D,D),bf16)]+[V((N1,128,128),bf16)]*2+[V((S,D),bf16)]*2
    sc+=[V((4,S+8,128),f32),V((4,N1*65,128),f32),V((4,N1*65,128),f32),V((8,N1*129,128),f32)]
    sc+=[V((D,D),bf16)]*2+[V((S+256,D),bf16)]*2+[V((D,S+256),bf16)]*2
    sc+=[pltpu.SemaphoreType.DMA((10,)),pltpu.SemaphoreType.DMA((8,)),pltpu.SemaphoreType.DMA((2,))]
    o=pl.pallas_call(kern,out_shape=jax.ShapeDtypeStruct((S,2*D),bf16),
      in_specs=[pl.BlockSpec(memory_space=pltpu.VMEM)]*4+[pl.BlockSpec(memory_space=pl.ANY)]*9,
      out_specs=pl.BlockSpec(memory_space=pl.ANY),scratch_shapes=sc,
      compiler_params=pltpu.CompilerParams(vmem_limit_bytes=110*2**20))(
      A_shift_k.T,A_ssm_D,F1c,G1c,A_q[0],A_k[0],A_v[0],A_ssm_k,B_x[0],B_wqkv,B_wo,F2c,G2c)
    return o[None]
```
